```python
import os as _os
_os.environ.setdefault("JAX_PLATFORMS", "cpu")
import jax
import jax.numpy as jnp

def _softmax(x, axis=-1):
    return jax.nn.softmax(x, axis=axis)
def _gelu(x):
    return jax.nn.gelu(x, approximate=True)
def _silu(x):
    return jax.nn.silu(x)
def _sigmoid(x):
    return jax.nn.sigmoid(x)
def _layernorm(x, axis=-1, eps=1e-5):
    m = jnp.mean(x, axis=axis, keepdims=True)
    v = jnp.var(x, axis=axis, keepdims=True)
    return (x - m) / jnp.sqrt(v + eps)
def _scatter_add(tgt, idx, src, axis=0):
    return tgt.at[idx].add(src)
def _segment_sum(src, seg, n):
    return jax.ops.segment_sum(src, seg, n)
class _Rng:
    def __init__(self, key):
        self._k = key
    def _next(self):
        self._k, sub = jax.random.split(self._k)
        return sub
    def normal(self, shape):
        return jax.random.normal(self._next(), shape, dtype=jnp.bfloat16)
    def randint(self, lo, hi, shape):
        return jax.random.randint(self._next(), shape, lo, hi, dtype=jnp.int32)
    def uniform(self, shape, lo=0.0, hi=1.0):
        return jax.random.uniform(self._next(), shape, jnp.bfloat16, lo, hi)
    def permutation(self, n):
        return jax.random.permutation(self._next(), n)


kernel_name = 'gated_mix__mha_block__mha_block__prompt'

def setup_inputs():
    _rng = _Rng(jax.random.key(int.from_bytes(__import__("os").urandom(4), "little")))
    _w = (lambda a: (lambda t: t.astype(jnp.bfloat16) if jnp.issubdtype(t.dtype, jnp.floating) else t)(jnp.asarray(a)))
    def _A_setup():
        B, S, D, H = 1, 2048, 448, 16
        return {
            "x": _w((lambda *s: _rng.normal(s) * 0.05)(B, S, D)),
            "wqkv": _w((lambda *s: _rng.normal(s) * 0.4)(D, 3 * D)),
            "wo": _w((lambda *s: _rng.normal(s) * 0.05)(D, D)),
        }
    _A_in = _A_setup()

    def _B_setup():
        B, S, D, H = 1, 2048, 448, 16
        return {
            "x": _w((lambda *s: _rng.normal(s) * 0.05)(B, S, D)),
            "wqkv": _w((lambda *s: _rng.normal(s) * 0.4)(D, 3 * D)),
            "wo": _w((lambda *s: _rng.normal(s) * 0.05)(D, D)),
        }
    _B_in = _B_setup()

    return {
        "A_x": _A_in["x"],
        "A_wqkv": _A_in["wqkv"],
        "A_wo": _A_in["wo"],
        "B_x": _B_in["x"],
        "B_wqkv": _B_in["wqkv"],
        "B_wo": _B_in["wo"],
        "gate_w": _w((lambda *s: _rng.normal(s) * 0.05)(448) * 16.0),
    }

def reference(A_x, A_wqkv, A_wo, B_x, B_wqkv, B_wo, gate_w):
    def _A_ref(x, wqkv, wo):
        B, S, D = x.shape
        H = 16
        Dh = D // H
        qkv = (lambda x, *d: x.transpose(*d))((x @ wqkv).reshape(B, S, 3, H, Dh), 2, 0, 3, 1, 4)
        q, k, v = qkv[0], qkv[1], qkv[2]
        scores = jnp.einsum("bhqd,bhkd->bhqk", q, k) * (Dh ** -0.5)
        p = _softmax(scores, axis=-1)
        o = jnp.einsum("bhqk,bhkd->bhqd", p, v)
        return (lambda x, *d: x.transpose(*d))(o, 0, 2, 1, 3).reshape(B, S, D) @ wo

    def _B_ref(x, wqkv, wo):
        B, S, D = x.shape
        H = 16
        Dh = D // H
        qkv = (lambda x, *d: x.transpose(*d))((x @ wqkv).reshape(B, S, 3, H, Dh), 2, 0, 3, 1, 4)
        q, k, v = qkv[0], qkv[1], qkv[2]
        scores = jnp.einsum("bhqd,bhkd->bhqk", q, k) * (Dh ** -0.5)
        p = _softmax(scores, axis=-1)
        o = jnp.einsum("bhqk,bhkd->bhqd", p, v)
        return (lambda x, *d: x.transpose(*d))(o, 0, 2, 1, 3).reshape(B, S, D) @ wo

    x = A_x
    g = _sigmoid((x * gate_w).sum(-1, keepdims=True))
    a = _A_ref(x, A_wqkv, A_wo)
    b = _B_ref(x, B_wqkv, B_wo)
    return g * a + (1 - g) * b
```

```python
import functools
import jax
import jax.numpy as jnp
import numpy as np
from jax.experimental import pallas as pl
from jax.experimental.pallas import tpu as pltpu

S, D, H, DH = 2048, 448, 16, 28
NH = 2 * H
BQ = 512
BK = 128
NQB = S // BQ
NB = NH * NQB
TB = 512
SCALE = float(DH ** -0.5 * 1.4426950408889634)
F32, BF16 = jnp.float32, jnp.bfloat16


def _nt(a, b):
    return jax.lax.dot_general(a, b, (((1,), (1,)), ((), ())), preferred_element_type=F32)


def _kernel(x_hbm, wa_hbm, wb_hbm, woa_hbm, wob_hbm, gw_ref, o_hbm,
            x_ref, w_ref, wo_ref, o_ref, in_sem, out_sem,
            wt_scr, wot_scr, k_scr, qt_scr, vt_scr, ot_scr, g_scr, s_scr, m_scr):
    NT = S // TB
    def x_copy(t):
        return pltpu.make_async_copy(x_hbm.at[:, pl.ds(t * TB, TB)], x_ref.at[:, pl.ds(t * TB, TB)], in_sem.at[t])
    def o_copy(t):
        return pltpu.make_async_copy(o_ref.at[:, pl.ds(t * TB, TB)], o_hbm.at[:, pl.ds(t * TB, TB)], out_sem.at[t])
    wa_cp = pltpu.make_async_copy(wa_hbm, w_ref.at[0], in_sem.at[NT])
    wb_cp = pltpu.make_async_copy(wb_hbm, w_ref.at[1], in_sem.at[NT + 1])
    woa_cp = pltpu.make_async_copy(woa_hbm, wo_ref.at[0], in_sem.at[NT + 2])
    wob_cp = pltpu.make_async_copy(wob_hbm, wo_ref.at[1], in_sem.at[NT + 3])
    wa_cp.start(); wb_cp.start()
    for t in range(NT):
        x_copy(t).start()
    woa_cp.start(); wob_cp.start()
    def tr(w):
        return w.astype(F32).T.astype(BF16)
    wa_cp.wait()
    for c in range(3):
        wt_scr[2 * c * D:(2 * c + 1) * D, :] = tr(w_ref[0, :, c * D:(c + 1) * D])
    wb_cp.wait()
    for c in range(3):
        wt_scr[(2 * c + 1) * D:(2 * c + 2) * D, :] = tr(w_ref[1, :, c * D:(c + 1) * D])
    wt_scr[6 * D:6 * D + 16, :] = jnp.broadcast_to(gw_ref[...].reshape(1, D), (16, D))

    def proj(t, _):
        t0 = pl.multiple_of(t * TB, TB)
        x_copy(t).wait()
        xb = x_ref[:, pl.ds(t0, TB)]
        r = jnp.dot(wt_scr[...], xb, preferred_element_type=F32)
        qt_scr[:, pl.ds(t0, TB)] = (r[0:2 * D] * SCALE).astype(BF16)
        for g in range(8):
            lo = 2 * D + 112 * g
            k_scr[g, pl.ds(t0, TB), :] = r[lo:lo + 128].T.astype(BF16)
        row = jax.lax.broadcasted_iota(jnp.int32, (4, TB), 0)
        tail = jnp.where(row == 0, 1.0, 0.0).astype(F32)
        for h in range(NH):
            v = r[4 * D + DH * h: 4 * D + DH * (h + 1)]
            vt_scr[32 * h:32 * h + 32, pl.ds(t0, TB)] = jnp.concatenate([v, tail], axis=0).astype(BF16)
        g_scr[:, pl.ds(t0, TB)] = jax.nn.sigmoid(r[6 * D:6 * D + 8])
        return _
    jax.lax.fori_loop(0, S // TB, proj, 0)

    def mk(it):
        h = it // NQB
        qb = it % NQB
        return h, pl.multiple_of(qb * BQ, BQ)

    def step(it_qk, slot_qk, it_pv, slot_pv):
        if it_qk is not None:
            h1, c1 = mk(it_qk)
            g1 = h1 // 4
            j1 = h1 % 4
            qg = qt_scr[pl.ds(pl.multiple_of(g1 * 112, 16), 112), pl.ds(c1, BQ)]
            rows = jax.lax.broadcasted_iota(jnp.int32, (112, BQ), 0)
            qg = jnp.where((rows >= j1 * DH) & (rows < j1 * DH + DH), qg, jnp.zeros_like(qg))
            qw = jnp.concatenate([qg, jnp.zeros((16, BQ), BF16)], axis=0)
        if it_pv is not None:
            h0, c0 = mk(it_pv)
            r0 = pl.multiple_of(h0 * 32, 32)
            m0 = m_scr[slot_pv]
        acc = jnp.zeros((32, BQ), F32)
        m = None
        for lo in range(0, S, BK):
            if it_qk is not None:
                sT = jnp.dot(k_scr[g1, lo:lo + BK, :], qw, preferred_element_type=F32)
                s_scr[slot_qk, lo:lo + BK, :] = sT
                mc = jnp.max(sT.reshape(BK // 8, 8, BQ), axis=0)
                m = mc if m is None else jnp.maximum(m, mc)
            if it_pv is not None:
                vT = vt_scr[pl.ds(r0, 32), lo:lo + BK]
                s0 = s_scr[slot_pv, lo:lo + BK, :]
                p = jnp.exp2((s0.reshape(BK // 8, 8, BQ) - m0[None]).reshape(BK, BQ)).astype(BF16)
                acc = acc + jnp.dot(vT, p, preferred_element_type=F32)
        if it_qk is not None:
            m_scr[slot_qk] = jnp.broadcast_to(jnp.max(m, axis=0, keepdims=True), (8, BQ))
        if it_pv is not None:
            l = acc[DH:DH + 1, :]
            ot_scr[pl.ds(r0, 32), pl.ds(c0, BQ)] = acc / l

    step(0, 0, None, None)

    def body(j, _):
        it = 2 * j
        step(it + 1, 1, it, 0)
        step(jnp.minimum(it + 2, NB - 1), 0, it + 1, 1)
        return _
    jax.lax.fori_loop(0, NB // 2, body, 0)

    woa_cp.wait(); wob_cp.wait()
    wot_scr[:, 0:D] = tr(wo_ref[0])
    wot_scr[:, D:2 * D] = tr(wo_ref[1])
    def outp(t, _):
        t0 = pl.multiple_of(t * TB, TB)
        g = g_scr[0:1, pl.ds(t0, TB)]
        parts = []
        for h in range(NH):
            o = ot_scr[32 * h:32 * h + DH, pl.ds(t0, TB)]
            parts.append(o * (g if h < H else 1.0 - g))
        oc = jnp.concatenate(parts, axis=0).astype(BF16)
        oT = jnp.dot(wot_scr[...], oc, preferred_element_type=F32)
        o_ref[:, pl.ds(t0, TB)] = oT.astype(o_ref.dtype)
        o_copy(t).start()
        return _
    jax.lax.fori_loop(0, S // TB, outp, 0)
    for t in range(NT):
        o_copy(t).wait()


@jax.jit
def pallas_gated_mix__mha_block__mha_block__prompt_kernel(A_x, A_wqkv, A_wo, B_x, B_wqkv, B_wo, gate_w):
    del B_x
    out = pl.pallas_call(
        _kernel,
        out_shape=jax.ShapeDtypeStruct((D, S), A_x.dtype),
        in_specs=[pl.BlockSpec(memory_space=pl.ANY)] * 5 + [pl.BlockSpec(memory_space=pltpu.VMEM)],
        out_specs=pl.BlockSpec(memory_space=pl.ANY),
        scratch_shapes=[
            pltpu.VMEM((D, S), BF16), pltpu.VMEM((2, D, 3 * D), BF16), pltpu.VMEM((2, D, D), BF16),
            pltpu.VMEM((D, S), BF16), pltpu.SemaphoreType.DMA((S // TB + 4,)), pltpu.SemaphoreType.DMA((S // TB,)),
            pltpu.VMEM((6 * D + 16, D), BF16),
            pltpu.VMEM((D, 2 * D), BF16),
            pltpu.VMEM((8, S, 128), BF16),
            pltpu.VMEM((2 * D, S), BF16),
            pltpu.VMEM((NH * 32, S), BF16),
            pltpu.VMEM((NH * 32, S), F32),
            pltpu.VMEM((8, S), F32),
            pltpu.VMEM((2, S, BQ), F32),
            pltpu.VMEM((2, 8, BQ), F32),
        ],
        compiler_params=pltpu.CompilerParams(vmem_limit_bytes=100 * 1024 * 1024),
    )(A_x.reshape(S, D).T, A_wqkv, B_wqkv, A_wo, B_wo, gate_w)
    return out.T.reshape(1, S, D)
```

```python
import jax
import jax.numpy as jnp
from jax.experimental import pallas as pl
from jax.experimental.pallas import tpu as pltpu

S, D, H, DH = 2048, 448, 16, 28
NH = 2 * H
BQ = 512
BK = 128
NC = S // BK
NQB = S // BQ
NB = NH * NQB
UNROLL = 14
TB = 512
NT = S // TB
SCALE = float(DH ** -0.5 * 1.4426950408889634)
F32, BF16 = jnp.float32, jnp.bfloat16


def _tn(a, b):
    return jax.lax.dot_general(a, b, (((0,), (0,)), ((), ())), preferred_element_type=F32)


def _kernel(x_hbm, wa_hbm, wb_hbm, woa_hbm, wob_hbm, gw_ref, o_hbm,
            x_ref, w_ref, wo_ref, o_ref, in_sem, out_sem,
            k_scr, qw_scr, vt_scr, ot_scr, g_scr, s_scr, m_scr, wot_scr):
    def x_copy(t):
        return pltpu.make_async_copy(x_hbm.at[:, pl.ds(t * TB, TB)], x_ref.at[:, pl.ds(t * TB, TB)], in_sem.at[t])

    def o_copy(t):
        return pltpu.make_async_copy(o_ref.at[:, pl.ds(t * TB, TB)], o_hbm.at[:, pl.ds(t * TB, TB)], out_sem.at[t])

    wa_cp = pltpu.make_async_copy(wa_hbm, w_ref.at[0], in_sem.at[NT])
    wb_cp = pltpu.make_async_copy(wb_hbm, w_ref.at[1], in_sem.at[NT + 1])
    woa_cp = pltpu.make_async_copy(woa_hbm, wo_ref.at[pl.ds(0, D)], in_sem.at[NT + 2])
    wob_cp = pltpu.make_async_copy(wob_hbm, wo_ref.at[pl.ds(D, D)], in_sem.at[NT + 3])
    wa_cp.start()
    x_copy(0).start()
    wa_cp.wait()
    x_copy(0).wait()
    wb_cp.start()
    for t in range(1, NT):
        x_copy(t).start()
    woa_cp.start()
    wob_cp.start()

    def proj(t, carry):
        t0 = pl.multiple_of(t * TB, TB)

        @pl.when(t > 0)
        def _wait_x():
            x_copy(t).wait()

        xb = x_ref[:, pl.ds(t0, TB)]
        rows112 = jax.lax.broadcasted_iota(jnp.int32, (4 * DH, TB), 0)
        row = jax.lax.broadcasted_iota(jnp.int32, (4, TB), 0)
        tail = jnp.where(row == 0, 1.0, 0.0).astype(F32)
        for blk in range(2):
            if blk == 1:
                @pl.when(t == 0)
                def _wait_wb():
                    wb_cp.wait()
            r = _tn(w_ref[blk], xb)
            q = (r[0:D] * SCALE).astype(BF16)
            for g in range(4):
                qg = q[112 * g:112 * (g + 1)]
                for i in range(4):
                    msk = (rows112 >= i * DH) & (rows112 < (i + 1) * DH)
                    qw_scr[blk * H + 4 * g + i, 0:112, pl.ds(t0, TB)] = jnp.where(msk, qg, jnp.zeros_like(qg))
                    qw_scr[blk * H + 4 * g + i, 112:128, pl.ds(t0, TB)] = jnp.zeros((16, TB), BF16)
            for g in range(4):
                lo = D + 112 * g
                k_scr[4 * blk + g, pl.ds(t0, TB), :] = r[lo:lo + 128].T.astype(BF16)
            for h in range(H):
                v = r[2 * D + DH * h: 2 * D + DH * (h + 1)]
                hh = blk * H + h
                vt_scr[32 * hh:32 * hh + 32, pl.ds(t0, TB)] = jnp.concatenate([v, tail], axis=0).astype(BF16)
        gl = jnp.dot(jnp.broadcast_to(gw_ref[...].reshape(1, D), (16, D)), xb, preferred_element_type=F32)
        g_scr[:, pl.ds(t0, TB)] = jax.nn.sigmoid(gl[0:8])
        return carry

    jax.lax.fori_loop(0, NT, proj, 0)

    def step(it_qk, slot_qk, it_pv, slot_pv):
        if it_qk is not None:
            h1 = it_qk // NQB
            c1 = pl.multiple_of((it_qk % NQB) * BQ, BQ)
            g1 = h1 // 4
            qw = qw_scr[h1, :, pl.ds(c1, BQ)]
        if it_pv is not None:
            r0 = pl.multiple_of((it_pv // NQB) * 32, 32)
            c0 = pl.multiple_of((it_pv % NQB) * BQ, BQ)
            m0 = m_scr[slot_pv]
        acc = None
        m = None
        for c in range(NC + 1):
            if it_qk is not None and c < NC:
                lo = c * BK
                sT = jnp.dot(k_scr[g1, lo:lo + BK, :], qw, preferred_element_type=F32)
                s_scr[slot_qk, lo:lo + BK, :] = sT
                mc = jnp.max(sT.reshape(BK // 8, 8, BQ), axis=0)
                m = mc if m is None else jnp.maximum(m, mc)
            if it_pv is not None and c >= 1:
                lo = (c - 1) * BK
                vT = vt_scr[pl.ds(r0, 32), lo:lo + BK]
                s0 = s_scr[slot_pv, lo:lo + BK, :]
                p = jnp.exp2((s0.reshape(BK // 8, 8, BQ) - m0[None]).reshape(BK, BQ)).astype(BF16)
                pv = jnp.dot(vT, p, preferred_element_type=F32)
                acc = pv if acc is None else acc + pv
        if it_qk is not None:
            m_scr[slot_qk] = jnp.broadcast_to(jnp.max(m, axis=0, keepdims=True), (8, BQ))
        if it_pv is not None:
            ot_scr[pl.ds(r0, 32), pl.ds(c0, BQ)] = acc

    woa_cp.wait()
    wob_cp.wait()
    wot_scr[...] = wo_ref[...].astype(F32).T.astype(BF16)
    step(0, 0, None, None)
    n_loop = (NB - 1) // UNROLL

    def body(j, carry):
        it = UNROLL * j
        for u in range(UNROLL):
            step(it + u + 1, (u + 1) % 2, it + u, u % 2)
        return carry

    jax.lax.fori_loop(0, n_loop, body, 0)
    for it in range(n_loop * UNROLL, NB):
        step(it + 1 if it + 1 < NB else None, (it + 1) % 2, it, it % 2)

    def outp(t, carry):
        t0 = pl.multiple_of(t * TB, TB)
        g = g_scr[0:1, pl.ds(t0, TB)]
        parts = []
        for h in range(NH):
            o = ot_scr[32 * h:32 * h + 32, pl.ds(t0, TB)]
            parts.append(o[0:DH] * ((g if h < H else 1.0 - g) / o[DH:DH + 1]))
        oc = jnp.concatenate(parts, axis=0).astype(BF16)
        o_ref[:, pl.ds(t0, TB)] = jnp.dot(wot_scr[...], oc, preferred_element_type=F32).astype(o_ref.dtype)
        o_copy(t).start()
        return carry

    jax.lax.fori_loop(0, NT, outp, 0)
    for t in range(NT):
        o_copy(t).wait()


@jax.jit
def pallas_gated_mix__mha_block__mha_block__prompt_kernel(A_x, A_wqkv, A_wo, B_x, B_wqkv, B_wo, gate_w):
    del B_x
    out_t = pl.pallas_call(
        _kernel,
        out_shape=jax.ShapeDtypeStruct((D, S), A_x.dtype),
        in_specs=[pl.BlockSpec(memory_space=pl.ANY)] * 5 + [pl.BlockSpec(memory_space=pltpu.VMEM)],
        out_specs=pl.BlockSpec(memory_space=pl.ANY),
        scratch_shapes=[
            pltpu.VMEM((D, S), BF16),
            pltpu.VMEM((2, D, 3 * D), BF16),
            pltpu.VMEM((2 * D, D), BF16),
            pltpu.VMEM((D, S), BF16),
            pltpu.SemaphoreType.DMA((NT + 4,)),
            pltpu.SemaphoreType.DMA((NT,)),
            pltpu.VMEM((8, S, 128), BF16),
            pltpu.VMEM((NH, 128, S), BF16),
            pltpu.VMEM((NH * 32, S), BF16),
            pltpu.VMEM((NH * 32, S), F32),
            pltpu.VMEM((8, S), F32),
            pltpu.VMEM((2, S, BQ), F32),
            pltpu.VMEM((2, 8, BQ), F32),
            pltpu.VMEM((D, 2 * D), BF16),
        ],
        compiler_params=pltpu.CompilerParams(vmem_limit_bytes=100 * 1024 * 1024),
    )(A_x.reshape(S, D).T, A_wqkv, B_wqkv, A_wo, B_wo, gate_w)
    return out_t.T.reshape(1, S, D)
```

```python
import jax
import jax.numpy as jnp
from jax.experimental import pallas as pl
from jax.experimental.pallas import tpu as pltpu

S, D, H, DH = 2048, 448, 16, 28
NH = 2 * H
BQ = 512
BK = 128
NC = S // BK
NQB = S // BQ
NB = NH * NQB
UNROLL = 14
TB = 512
NT = S // TB
SCALE = float(DH ** -0.5 * 1.4426950408889634)
F32, BF16 = jnp.float32, jnp.bfloat16


def _tn(a, b):
    return jax.lax.dot_general(a, b, (((0,), (0,)), ((), ())), preferred_element_type=F32)


def _kernel(x_hbm, wa_hbm, wb_hbm, woa_hbm, wob_hbm, gw_ref, o_hbm,
            x_ref, w_ref, wo_ref, o_ref, in_sem, out_sem,
            k_scr, qw_scr, vt_scr, ot_scr, g_scr, s_scr, m_scr, wot_scr):
    def x_copy(t):
        return pltpu.make_async_copy(x_hbm.at[:, pl.ds(t * TB, TB)], x_ref.at[:, pl.ds(t * TB, TB)], in_sem.at[t])

    def o_copy(t):
        return pltpu.make_async_copy(o_ref.at[:, pl.ds(t * TB, TB)], o_hbm.at[:, pl.ds(t * TB, TB)], out_sem.at[t])

    wa_cp = pltpu.make_async_copy(wa_hbm, w_ref.at[0], in_sem.at[NT])
    wb_cp = pltpu.make_async_copy(wb_hbm, w_ref.at[1], in_sem.at[NT + 1])
    woa_cp = pltpu.make_async_copy(woa_hbm, wo_ref.at[pl.ds(0, D)], in_sem.at[NT + 2])
    wob_cp = pltpu.make_async_copy(wob_hbm, wo_ref.at[pl.ds(D, D)], in_sem.at[NT + 3])
    wa_cp.start()
    x_copy(0).start()
    wa_cp.wait()
    x_copy(0).wait()
    wb_cp.start()
    for t in range(1, NT):
        x_copy(t).start()
    woa_cp.start()
    wob_cp.start()

    rows112 = jax.lax.broadcasted_iota(jnp.int32, (4 * DH, TB), 0)
    row = jax.lax.broadcasted_iota(jnp.int32, (4, TB), 0)
    tail = jnp.where(row == 0, 1.0, 0.0).astype(F32)

    def proj(t, blk):
        t0 = t * TB if isinstance(t, int) else pl.multiple_of(t * TB, TB)
        xb = x_ref[:, pl.ds(t0, TB)]
        r = _tn(w_ref[blk], xb)
        q = (r[0:D] * SCALE).astype(BF16)
        for g in range(4):
            qg = q[112 * g:112 * (g + 1)]
            for i in range(4):
                msk = (rows112 >= i * DH) & (rows112 < (i + 1) * DH)
                qw_scr[blk * H + 4 * g + i, 0:112, pl.ds(t0, TB)] = jnp.where(msk, qg, jnp.zeros_like(qg))
                qw_scr[blk * H + 4 * g + i, 112:128, pl.ds(t0, TB)] = jnp.zeros((16, TB), BF16)
        for g in range(4):
            lo = D + 112 * g
            k_scr[4 * blk + g, pl.ds(t0, TB), :] = r[lo:lo + 128].T.astype(BF16)
        for h in range(H):
            v = r[2 * D + DH * h: 2 * D + DH * (h + 1)]
            hh = blk * H + h
            vt_scr[32 * hh:32 * hh + 32, pl.ds(t0, TB)] = jnp.concatenate([v, tail], axis=0).astype(BF16)
        if blk == 0:
            gl = jnp.dot(jnp.broadcast_to(gw_ref[...].reshape(1, D), (16, D)), xb, preferred_element_type=F32)
            g_scr[:, pl.ds(t0, TB)] = jax.nn.sigmoid(gl[0:8])

    proj(0, 0)
    wb_cp.wait()

    def proj_body(t, carry):
        x_copy(t).wait()
        proj(t - 1, 1)
        proj(t, 0)
        return carry

    jax.lax.fori_loop(1, NT, proj_body, 0)
    proj(NT - 1, 1)

    def step(it_qk, slot_qk, it_pv, slot_pv):
        if it_qk is not None:
            h1 = it_qk // NQB
            c1 = pl.multiple_of((it_qk % NQB) * BQ, BQ)
            g1 = h1 // 4
            qw = qw_scr[h1, :, pl.ds(c1, BQ)]
        if it_pv is not None:
            r0 = pl.multiple_of((it_pv // NQB) * 32, 32)
            c0 = pl.multiple_of((it_pv % NQB) * BQ, BQ)
            m0 = m_scr[slot_pv]
        acc = None
        m = None
        for c in range(NC + 1):
            if it_qk is not None and c < NC:
                lo = c * BK
                sT = jnp.dot(k_scr[g1, lo:lo + BK, :], qw, preferred_element_type=F32)
                s_scr[slot_qk, lo:lo + BK, :] = sT
                mc = jnp.max(sT.reshape(BK // 8, 8, BQ), axis=0)
                m = mc if m is None else jnp.maximum(m, mc)
            if it_pv is not None and c >= 1:
                lo = (c - 1) * BK
                vT = vt_scr[pl.ds(r0, 32), lo:lo + BK]
                s0 = s_scr[slot_pv, lo:lo + BK, :]
                p = jnp.exp2((s0.reshape(BK // 8, 8, BQ) - m0[None]).reshape(BK, BQ)).astype(BF16)
                pv = jnp.dot(vT, p, preferred_element_type=F32)
                acc = pv if acc is None else acc + pv
        if it_qk is not None:
            m_scr[slot_qk] = jnp.broadcast_to(jnp.max(m, axis=0, keepdims=True), (8, BQ))
        if it_pv is not None:
            ot_scr[pl.ds(r0, 32), pl.ds(c0, BQ)] = acc

    woa_cp.wait()
    wob_cp.wait()
    wot_scr[...] = wo_ref[...].astype(F32).T.astype(BF16)
    step(0, 0, None, None)
    n_loop = (NB - 1) // UNROLL

    def body(j, carry):
        it = UNROLL * j
        for u in range(UNROLL):
            step(it + u + 1, (u + 1) % 2, it + u, u % 2)
        return carry

    jax.lax.fori_loop(0, n_loop, body, 0)
    for it in range(n_loop * UNROLL, NB):
        step(it + 1 if it + 1 < NB else None, (it + 1) % 2, it, it % 2)

    def outp(t, carry):
        t0 = pl.multiple_of(t * TB, TB)
        g = g_scr[0:1, pl.ds(t0, TB)]
        parts = []
        for h in range(NH):
            o = ot_scr[32 * h:32 * h + 32, pl.ds(t0, TB)]
            parts.append(o[0:DH] * ((g if h < H else 1.0 - g) / o[DH:DH + 1]))
        oc = jnp.concatenate(parts, axis=0).astype(BF16)
        o_ref[:, pl.ds(t0, TB)] = jnp.dot(wot_scr[...], oc, preferred_element_type=F32).astype(o_ref.dtype)
        o_copy(t).start()
        return carry

    jax.lax.fori_loop(0, NT, outp, 0)
    for t in range(NT):
        o_copy(t).wait()


@jax.jit
def pallas_gated_mix__mha_block__mha_block__prompt_kernel(A_x, A_wqkv, A_wo, B_x, B_wqkv, B_wo, gate_w):
    del B_x
    out_t = pl.pallas_call(
        _kernel,
        out_shape=jax.ShapeDtypeStruct((D, S), A_x.dtype),
        in_specs=[pl.BlockSpec(memory_space=pl.ANY)] * 5 + [pl.BlockSpec(memory_space=pltpu.VMEM)],
        out_specs=pl.BlockSpec(memory_space=pl.ANY),
        scratch_shapes=[
            pltpu.VMEM((D, S), BF16),
            pltpu.VMEM((2, D, 3 * D), BF16),
            pltpu.VMEM((2 * D, D), BF16),
            pltpu.VMEM((D, S), BF16),
            pltpu.SemaphoreType.DMA((NT + 4,)),
            pltpu.SemaphoreType.DMA((NT,)),
            pltpu.VMEM((8, S, 128), BF16),
            pltpu.VMEM((NH, 128, S), BF16),
            pltpu.VMEM((NH * 32, S), BF16),
            pltpu.VMEM((NH * 32, S), F32),
            pltpu.VMEM((8, S), F32),
            pltpu.VMEM((2, S, BQ), F32),
            pltpu.VMEM((2, 8, BQ), F32),
            pltpu.VMEM((D, 2 * D), BF16),
        ],
        compiler_params=pltpu.CompilerParams(vmem_limit_bytes=100 * 1024 * 1024),
    )(A_x.reshape(S, D).T, A_wqkv, B_wqkv, A_wo, B_wo, gate_w)
    return out_t.T.reshape(1, S, D)
```
